```python
import os as _os
_os.environ.setdefault("JAX_PLATFORMS", "cpu")
import jax
import jax.numpy as jnp

def _softmax(x, axis=-1):
    return jax.nn.softmax(x, axis=axis)
def _gelu(x):
    return jax.nn.gelu(x, approximate=True)
def _silu(x):
    return jax.nn.silu(x)
def _sigmoid(x):
    return jax.nn.sigmoid(x)
def _layernorm(x, axis=-1, eps=1e-5):
    m = jnp.mean(x, axis=axis, keepdims=True)
    v = jnp.var(x, axis=axis, keepdims=True)
    return (x - m) / jnp.sqrt(v + eps)
def _scatter_add(tgt, idx, src, axis=0):
    return tgt.at[idx].add(src)
def _segment_sum(src, seg, n):
    return jax.ops.segment_sum(src, seg, n)
class _Rng:
    def __init__(self, key):
        self._k = key
    def _next(self):
        self._k, sub = jax.random.split(self._k)
        return sub
    def normal(self, shape):
        return jax.random.normal(self._next(), shape, dtype=jnp.bfloat16)
    def randint(self, lo, hi, shape):
        return jax.random.randint(self._next(), shape, lo, hi, dtype=jnp.int32)
    def uniform(self, shape, lo=0.0, hi=1.0):
        return jax.random.uniform(self._next(), shape, jnp.bfloat16, lo, hi)
    def permutation(self, n):
        return jax.random.permutation(self._next(), n)


kernel_name = 'gated_mix__grouped_kv_mqa__ssm_conv_s5__prompt'

def setup_inputs():
    _rng = _Rng(jax.random.key(int.from_bytes(__import__("os").urandom(4), "little")))
    _w = (lambda a: (lambda t: t.astype(jnp.bfloat16) if jnp.issubdtype(t.dtype, jnp.floating) else t)(jnp.asarray(a)))
    def _A_setup():
        B, S, D, H = 1, 2048, 512, 32
        Dh = D // H
        return {
            "x": _w((lambda *s: _rng.normal(s) * 0.05)(B, S, D)),
            "wq": _w((lambda *s: _rng.normal(s) * 1.6)(D, H * Dh)),
            "wk": _w((lambda *s: _rng.normal(s) * 1.6)(D, Dh)),
            "wv": _w((lambda *s: _rng.normal(s) * 0.05)(D, Dh)),
            "wo": _w((lambda *s: _rng.normal(s) * 0.05)(H * Dh, D)),
        }
    _A_in = _A_setup()

    def _B_setup():
        B, S, D = 1, 2048, 512
        P = D
        Lambda_re = -0.5 * jnp.exp((lambda *s: _rng.normal(s) * 0.4)(P))
        Lambda_im = (lambda *s: _rng.normal(s) * 0.4)(P) * 1.0
        B_re = (lambda *s: _rng.normal(s) * 0.4)(P, D) * (D ** -0.5)
        B_im = (lambda *s: _rng.normal(s) * 0.4)(P, D) * (D ** -0.5)
        C_re = (lambda *s: _rng.normal(s) * 0.4)(D, P) * (P ** -0.5)
        C_im = (lambda *s: _rng.normal(s) * 0.4)(D, P) * (P ** -0.5)
        log_dt = (lambda *s: _rng.normal(s) * 0.4)(P) * 0.3 - 2.0
        Dskip = (lambda *s: _rng.normal(s) * 0.4)(D)
        return {
            "x": _w((lambda *s: _rng.normal(s) * 0.05)(B, S, D)),
            "Lambda_re": _w(Lambda_re),
            "Lambda_im": _w(Lambda_im),
            "B_re": _w(B_re),
            "B_im": _w(B_im),
            "C_re": _w(C_re),
            "C_im": _w(C_im),
            "log_dt": _w(log_dt),
            "Dskip": _w(Dskip),
        }
    _B_in = _B_setup()

    return {
        "A_x": _A_in["x"],
        "A_wq": _A_in["wq"],
        "A_wk": _A_in["wk"],
        "A_wv": _A_in["wv"],
        "A_wo": _A_in["wo"],
        "B_x": _B_in["x"],
        "B_Lambda_re": _B_in["Lambda_re"],
        "B_Lambda_im": _B_in["Lambda_im"],
        "B_B_re": _B_in["B_re"],
        "B_B_im": _B_in["B_im"],
        "B_C_re": _B_in["C_re"],
        "B_C_im": _B_in["C_im"],
        "B_log_dt": _B_in["log_dt"],
        "B_Dskip": _B_in["Dskip"],
        "gate_w": _w((lambda *s: _rng.normal(s) * 0.05)(512) * 16.0),
    }

def reference(A_x, A_wq, A_wk, A_wv, A_wo, B_x, B_Lambda_re, B_Lambda_im, B_B_re, B_B_im, B_C_re, B_C_im, B_log_dt, B_Dskip, gate_w):
    def _A_ref(x, wq, wk, wv, wo):
        B, S, D = x.shape
        H = 32
        Dh = D // H
        q = (lambda x, *d: x.transpose(*d))((x @ wq).reshape(B, S, H, Dh), 0, 2, 1, 3)
        k = x @ wk
        v = x @ wv
        scores = jnp.einsum("bhqd,bkd->bhqk", q, k) * (Dh ** -0.5)
        p = _softmax(scores, axis=-1)
        o = jnp.einsum("bhqk,bkd->bhqd", p, v)
        return (lambda x, *d: x.transpose(*d))(o, 0, 2, 1, 3).reshape(B, S, H * Dh) @ wo

    def _B_ref(x, Lambda_re, Lambda_im, B_re, B_im, C_re, C_im, log_dt, Dskip):
        Bsz, L, H = x.shape
        Lam = Lambda_re + 1j * Lambda_im
        Bmat = B_re + 1j * B_im
        Cmat = C_re + 1j * C_im
        dt = jnp.exp(log_dt)
        Lam_bar = jnp.exp(dt * Lam)
        B_bar = ((Lam_bar - 1.0) / Lam)[:, None] * Bmat
        Bu = jnp.einsum("bld,pd->blp", x + 0j, B_bar)
        h = jnp.zeros_like(Bu[:, 0, :])
        hs = []
        for t in range(L):
            h = Lam_bar[None, :] * h + Bu[:, t, :]
            hs.append(h)
        hseq = jnp.stack(hs, 1)
        y = 2.0 * jnp.einsum("blp,dp->bld", hseq, Cmat).real + x * Dskip[None, None, :]
        return y

    x = A_x
    g = _sigmoid((x * gate_w).sum(-1, keepdims=True))
    a = _A_ref(x, A_wq, A_wk, A_wv, A_wo)
    b = _B_ref(x, B_Lambda_re, B_Lambda_im, B_B_re, B_B_im, B_C_re, B_C_im, B_log_dt, B_Dskip)
    return g * a + (1 - g) * b
```

```python
import functools
import jax
import jax.numpy as jnp
from jax import lax
import jax.experimental.pallas as pl
import jax.experimental.pallas.tpu as pltpu

S = 2048
D = 512
H = 32
DH = 16
P = 512
BQ = 512
CK = 128
NIT = 4
LAG = 2
LOG2E = 1.4426950408889634
QSCALE = (DH ** -0.5) * LOG2E

bf16 = jnp.bfloat16
f32 = jnp.float32
u32 = jnp.uint32

NT = (((1,), (1,)), ((), ()))
TN = (((0,), (0,)), ((), ()))


def _cmul(ar, ai, br, bi):
    return ar * br - ai * bi, ar * bi + ai * br


def _kernel(x_ref, wq_ref, wkT_ref, wvT_ref, wo_ref, lre_ref, lim_ref, bre_ref, bim_ref,
            cre_ref, cim_ref, ldt_ref, dskip_ref, gate_ref, o_ref,
            qa_ref, k_ref, vt_ref, g_ref, bu_ref, h_ref, ot_ref, cst_ref):
    gate16 = jnp.broadcast_to(gate_ref[...].reshape(1, D), (16, D))
    wT = jnp.concatenate([wq_ref[...].T, wkT_ref[...], wvT_ref[...], gate16], axis=0)
    kts = []
    for j in range(S // 512):
        cs = slice(j * 512, (j + 1) * 512)
        r = lax.dot_general(wT, x_ref[cs, :], NT, preferred_element_type=f32)
        q = (r[:D] * QSCALE).astype(bf16)
        for h in range(H):
            qh = q[h * DH:(h + 1) * DH]
            qf = qh.astype(f32)
            nrm = jnp.sqrt(jnp.sum(qf * qf, axis=0, keepdims=True))
            qa_ref[h * 32:h * 32 + 16, cs] = qh
            qa_ref[h * 32 + 16:h * 32 + 32, cs] = jnp.broadcast_to(-nrm, (16, 512)).astype(bf16)
        kts.append(r[D:D + 16].astype(bf16).astype(f32))
        vt_ref[:, cs] = pltpu.bitcast(r[D + 16:D + 32].astype(bf16), u32)
        gt = jax.nn.sigmoid(r[D + 32:D + 48])
        g_ref[cs, :] = jnp.concatenate([gt] * 8, axis=0).T
    kt = jnp.concatenate(kts, axis=1)
    kn2 = jnp.sum(kt * kt, axis=0, keepdims=True)
    kmax = jnp.sqrt(jnp.max(kn2, axis=1, keepdims=True))
    krow = jnp.broadcast_to(kmax * (1.0 / 16.0), (16, S))
    T = jnp.concatenate([kt, krow, jnp.zeros((96, S), f32)], axis=0)
    k_ref[...] = pltpu.bitcast(T.T.astype(bf16), u32)

    lre = lre_ref[...].reshape(1, P).astype(f32)
    lim = lim_ref[...].reshape(1, P).astype(f32)
    dt = jnp.exp(ldt_ref[...].reshape(1, P).astype(f32)).astype(bf16).astype(f32)
    kk = (lax.broadcasted_iota(jnp.int32, (8, P), 0) + 1).astype(f32)
    mag = jnp.exp(kk * (dt * lre))
    ang = kk * (dt * lim)
    pwr = mag * jnp.cos(ang)
    pwi = mag * jnp.sin(ang)
    row = lax.broadcasted_iota(jnp.int32, (8, P), 0)
    l1r, l1i = pwr[0:1], pwi[0:1]
    den = 1.0 / (lre * lre + lim * lim)
    nr = l1r - 1.0
    cfr = (nr * lre + l1i * lim) * den
    cfi = (l1i * lre - nr * lim) * den
    cst_ref[0] = jnp.broadcast_to(cfr, (8, P))
    cst_ref[1] = jnp.broadcast_to(cfi, (8, P))
    for n, (sh, src) in enumerate(((1, 0), (2, 1), (4, 3))):
        cst_ref[2 + 2 * n] = jnp.where(row >= sh, jnp.broadcast_to(pwr[src:src + 1], (8, P)), 0.0)
        cst_ref[3 + 2 * n] = jnp.where(row >= sh, jnp.broadcast_to(pwi[src:src + 1], (8, P)), 0.0)
    cst_ref[8] = pwr
    cst_ref[9] = pwi

    bcat = jnp.concatenate([bre_ref[...], bim_ref[...]], axis=0)

    def b_body(i, c):
        rs = pl.ds(pl.multiple_of(i * 256, 256), 256)
        bu_ref[rs, :] = lax.dot_general(x_ref[rs, :], bcat, NT, preferred_element_type=f32)
        return c
    lax.fori_loop(0, S // 256, b_body, 0)

    TS = 64

    def scan_chunk(t0, carry):
        new_carry = []
        rs = pl.ds(t0, TS)
        for gi in range(P // 128):
            ls = slice(gi * 128, (gi + 1) * 128)
            hs = slice(P + gi * 128, P + (gi + 1) * 128)
            br = bu_ref[rs, ls].reshape(TS // 8, 8, 128)
            bi = bu_ref[rs, hs].reshape(TS // 8, 8, 128)
            ur, ui = _cmul(cst_ref[0, :, ls][None], cst_ref[1, :, ls][None], br, bi)
            for n, sh in enumerate((1, 2, 4)):
                rr = pltpu.roll(ur, sh, 1)
                ri = pltpu.roll(ui, sh, 1)
                tr, ti = _cmul(cst_ref[2 + 2 * n, :, ls][None], cst_ref[3 + 2 * n, :, ls][None], rr, ri)
                ur = ur + tr
                ui = ui + ti
            pr, pi = cst_ref[8, :, ls], cst_ref[9, :, ls]
            cr, ci = carry[gi]
            outr, outi = [], []
            for b in range(TS // 8):
                tr, ti = _cmul(pr, pi, cr, ci)
                hr = ur[b] + tr
                hi = ui[b] + ti
                cr = jnp.broadcast_to(hr[7:8], (8, 128))
                ci = jnp.broadcast_to(hi[7:8], (8, 128))
                outr.append(hr)
                outi.append(hi)
            h_ref[rs, ls] = (jnp.concatenate(outr, axis=0) * 2.0).astype(bf16)
            h_ref[rs, hs] = (jnp.concatenate(outi, axis=0) * -2.0).astype(bf16)
            new_carry.append((cr, ci))
        return tuple(new_carry)

    z = jnp.zeros((8, 128), f32)
    lax.fori_loop(0, S // TS, lambda i, c: scan_chunk(pl.multiple_of(i * TS, TS), c),
                  tuple((z, z) for _ in range(P // 128)))

    NQ = S // BQ
    NI = H * NQ
    NC = S // CK

    def ld_k(c):
        return pltpu.bitcast(k_ref[c * CK // 2:(c + 1) * CK // 2, :], bf16)[:, :32]

    def ld_vt(c):
        return pltpu.bitcast(vt_ref[:, c * CK:(c + 1) * CK], bf16)

    def attn_body(ii, okv):
        base = ii * NIT
        qts = {}

        def getq(r):
            if r not in qts:
                i = base + r
                h = i // NQ
                j = i % NQ
                qts[r] = qa_ref[pl.ds(pl.multiple_of(h * 32, 32), 32), pl.ds(pl.multiple_of(j * BQ, BQ), BQ)]
            return qts[r]
        pend = {}
        l = acc = None
        for g in range(NIT * NC + LAG):
            if g < NIT * NC:
                r, c = g // NC, g % NC
                pend[g] = jnp.dot(ld_k(c), getq(r), preferred_element_type=f32)
            gp = g - LAG
            if gp >= 0:
                r, c = gp // NC, gp % NC
                p = jnp.exp2(pend.pop(gp))
                ls = jnp.sum(p.reshape(CK // 8, 8, BQ), axis=0)
                l = ls if l is None else l + ls
                o = jnp.dot(ld_vt(c), p.astype(bf16), preferred_element_type=f32)
                acc = o if acc is None else acc + o
                if c == NC - 1:
                    i = base + r
                    h = i // NQ
                    j = i % NQ
                    lsum = jnp.sum(l, axis=0, keepdims=True)
                    okv = jnp.minimum(okv, jnp.where((lsum > 2.0 ** -50) & (lsum < 2.0 ** 50), 1.0, 0.0))
                    ot_ref[pl.ds(pl.multiple_of(h * 16, 16), 16), pl.ds(pl.multiple_of(j * BQ, BQ), BQ)] = (
                        acc * (1.0 / lsum)).astype(bf16)
                    l = acc = None
        return okv
    okv = lax.fori_loop(0, NI // NIT, attn_body, jnp.ones((1, BQ), f32))

    @pl.when(jnp.min(okv) < 0.5)
    def _fallback():
        def fb(i, c):
            h = i // (S // 128)
            j = i % (S // 128)
            qt = qa_ref[pl.ds(pl.multiple_of(h * 32, 32), 16), pl.ds(pl.multiple_of(j * 128, 128), 128)]
            kf = pltpu.bitcast(k_ref[...], bf16)[:, :16]
            s = jnp.dot(kf, qt, preferred_element_type=f32)
            m = jnp.max(s, axis=0, keepdims=True)
            p = jnp.exp2(s - m)
            l = jnp.sum(p, axis=0, keepdims=True)
            o = jnp.dot(pltpu.bitcast(vt_ref[...], bf16), p.astype(bf16), preferred_element_type=f32)
            ot_ref[pl.ds(pl.multiple_of(h * 16, 16), 16), pl.ds(pl.multiple_of(j * 128, 128), 128)] = (
                o * (1.0 / l)).astype(bf16)
            return c
        lax.fori_loop(0, H * (S // 128), fb, 0)

    ccat = jnp.concatenate([cre_ref[...], cim_ref[...]], axis=1)
    wo = wo_ref[...]
    dskip = dskip_ref[...].reshape(1, D).astype(f32)
    RF = 256

    def f_body(i, c):
        rs = pl.ds(pl.multiple_of(i * RF, RF), RF)
        yb = lax.dot_general(h_ref[rs, :], ccat, NT, preferred_element_type=f32)
        ya = lax.dot_general(ot_ref[:, rs], wo, TN, preferred_element_type=f32)
        g1 = g_ref[rs, :]
        g = jnp.concatenate([g1] * 4, axis=1)
        yb = yb + x_ref[rs, :].astype(f32) * dskip
        o_ref[rs, :] = g * ya + (1.0 - g) * yb
        return c
    lax.fori_loop(0, S // RF, f_body, 0)


@jax.jit
def pallas_gated_mix__grouped_kv_mqa__ssm_conv_s5__prompt_kernel(
    A_x, A_wq, A_wk, A_wv, A_wo, B_x, B_Lambda_re, B_Lambda_im, B_B_re, B_B_im, B_C_re, B_C_im,
    B_log_dt, B_Dskip, gate_w,
):
    del B_x
    out = pl.pallas_call(
        _kernel,
        out_shape=jax.ShapeDtypeStruct((S, D), f32),
        scratch_shapes=[
            pltpu.VMEM((H * 32, S), bf16),
            pltpu.VMEM((S // 2, 128), u32),
            pltpu.VMEM((8, S), u32),
            pltpu.VMEM((S, 128), f32),
            pltpu.VMEM((S, 2 * P), f32),
            pltpu.VMEM((S, 2 * P), bf16),
            pltpu.VMEM((D, S), bf16),
            pltpu.VMEM((10, 8, P), f32),
        ],
        compiler_params=pltpu.CompilerParams(vmem_limit_bytes=100 * 2 ** 20),
        name="gmix",
    )(A_x.reshape(S, D), A_wq, A_wk.T, A_wv.T, A_wo, B_Lambda_re, B_Lambda_im, B_B_re, B_B_im,
      B_C_re, B_C_im, B_log_dt, B_Dskip, gate_w)
    return out.reshape(1, S, D)
```

```python
import jax
import jax.numpy as jnp
from jax import lax
import jax.experimental.pallas as pl
import jax.experimental.pallas.tpu as pltpu

S = 2048
D = 512
H = 32
DH = 16
P = 512
BQ = 512
CK = 128
HPI = 2
LAG = 2
XB = 512
FCH = (256,) * 7 + (128, 64, 64)

LOG2E = 1.4426950408889634
QSCALE = (DH ** -0.5) * LOG2E
L_LO = 2.0 ** -64
L_HI = 2.0 ** 12
V_UP = 2.0 ** 40

bf16 = jnp.bfloat16
f32 = jnp.float32
u32 = jnp.uint32

NT = (((1,), (1,)), ((), ()))
TN = (((0,), (0,)), ((), ()))

NQ = S // BQ
NCA = S // CK
NC = NCA - 1
NIT = NQ * HPI
NLOOP = H // HPI
NG = P // 128
TS = S * NG // NLOOP
NP = 32

T_KC = 0
T_ANC = 1
T_KB = 2
T_PVB = T_KB + 256
PPI = 36
T_END = T_PVB + (NIT // 2) * PPI

CHT = 136
PSP = NIT * NC * CHT / (NP * NIT)
FREE = 2
SSP = NIT * NC * CHT / (TS // 8)
SOFF = 112


def _cmul(ar, ai, br, bi):
    return ar * br - ai * bi, ar * bi + ai * br


def _slot_of(t):
    g = int(t // CHT)
    return g, min(int((t - g * CHT) // 8), 15)


def _kernel(x_hbm, wq_hbm, wkT_hbm, wvT_hbm, wo_hbm, lre_hbm, lim_hbm, bre_hbm, bim_hbm,
            cre_hbm, cim_hbm, ldt_hbm, dskip_hbm, gate_hbm, o_hbm,
            x_ref, wq_ref, wkT_ref, wvT_ref, wo_ref, lre_ref, lim_ref, bre_ref, bim_ref,
            cre_ref, cim_ref, ldt_ref, dskip_ref, gate_ref, o_ref,
            qa_ref, qf_ref, k_ref, vt_ref, bu_ref, h_ref, ot_ref, cst_ref, ka_refs, car_ref, ok_ref, pc_ref,
            isem, osem):
    def cp(src, dst, n):
        return pltpu.make_async_copy(src, dst, isem.at[n])
    x_cps = [cp(x_hbm.at[pl.ds(j * XB, XB)], x_ref.at[pl.ds(j * XB, XB)], j) for j in range(S // XB)]
    wq_cp = cp(wq_hbm, wq_ref, 4)
    small = [cp(wkT_hbm, wkT_ref, 5), cp(wvT_hbm, wvT_ref, 6),
             cp(lre_hbm, lre_ref, 8), cp(lim_hbm, lim_ref, 9), cp(ldt_hbm, ldt_ref, 10)]
    b_cps = [cp(bre_hbm, bre_ref, 12), cp(bim_hbm, bim_ref, 13)]
    c_cps = [cp(cre_hbm, cre_ref, 14), cp(cim_hbm, cim_ref, 15), cp(wo_hbm, wo_ref, 16),
             cp(dskip_hbm, dskip_ref, 11), cp(gate_hbm, gate_ref, 7)]

    def start(cs):
        for c in cs:
            c.start()

    def wait(cs):
        for c in cs:
            c.wait()

    start(small + [wq_cp] + x_cps + b_cps)
    wait(small + [wq_cp])

    wT = jnp.concatenate([wkT_ref[...], wvT_ref[...], wq_ref[...].T], axis=0)
    kts = []

    def proj(j):
        return lax.dot_general(wT, x_ref[j * XB:(j + 1) * XB, :], NT, preferred_element_type=f32)

    def post(j, r):
        cs = slice(j * XB, (j + 1) * XB)
        qs = r[2 * DH:] * QSCALE
        for h in range(H):
            qf = qs[h * DH:(h + 1) * DH]
            n2 = jnp.sum(qf * qf, axis=0, keepdims=True)
            nn = n2 * lax.rsqrt(n2 + 1e-30) * (-1.0 - 2.0 ** -7)
            qh = qf.astype(bf16)
            nh = jnp.broadcast_to(nn, (16, XB)).astype(bf16)
            qa_ref[h * 32:h * 32 + 16, cs] = qh
            qa_ref[h * 32 + 16:h * 32 + 32, cs] = nh
            qf_ref[h, 0:16, cs] = qh.astype(f32)
            qf_ref[h, 16:24, cs] = nh.astype(f32)[0:8]
        kts.append(r[:DH].astype(bf16).astype(f32))
        vt_ref[:, cs] = pltpu.bitcast((r[DH:2 * DH] * V_UP).astype(bf16), u32)

    def ssm_consts():
        lre = lre_ref[...].reshape(1, P).astype(f32)
        lim = lim_ref[...].reshape(1, P).astype(f32)
        dt = jnp.exp(ldt_ref[...].reshape(1, P).astype(f32)).astype(bf16).astype(f32)
        row = lax.broadcasted_iota(jnp.int32, (8, P), 0)
        kk = jnp.where(row == 0, 1, jnp.where(row == 1, 2, 4)).astype(f32)
        mag = jnp.exp(kk * (dt * lre))
        ang = kk * (dt * lim)
        pwr = mag * jnp.cos(ang)
        pwi = mag * jnp.sin(ang)
        l1r, l1i = pwr[0:1], pwi[0:1]
        den = 2.0 / (lre * lre + lim * lim)
        nr = l1r - 1.0
        cfr = (nr * lre + l1i * lim) * den
        cfi = (l1i * lre - nr * lim) * den
        consts = [
            jnp.where(row == 0, jnp.broadcast_to(l1r, (8, P)), 0.0),
            jnp.where(row == 0, jnp.broadcast_to(-l1i, (8, P)), 0.0),
        ]
        for sh, src in ((1, 0), (2, 1), (4, 2)):
            consts.append(jnp.where(row >= sh, jnp.broadcast_to(pwr[src:src + 1], (8, P)), 0.0))
            consts.append(jnp.where(row >= sh, jnp.broadcast_to(-pwi[src:src + 1], (8, P)), 0.0))
        for n, cv in enumerate(consts):
            for gi in range(NG):
                cst_ref[n * NG + gi] = cv[:, gi * 128:(gi + 1) * 128]
        cfT = jnp.concatenate([jnp.broadcast_to(cfr, (64, P)), jnp.broadcast_to(cfi, (64, P))], axis=0).T
        return cfT[:, 0:1], cfT[:, 64:65]

    crc, cic = ssm_consts()
    wait(x_cps[:1])
    post(0, proj(0))
    wait(x_cps[1:3])
    post(1, proj(1))
    post(2, proj(2))
    wait(x_cps[3:] + b_cps)
    start(c_cps)
    r3 = proj(3)

    br = bre_ref[...].astype(f32)
    bi = bim_ref[...].astype(f32)
    bcat = jnp.concatenate([(crc * br - cic * bi).astype(bf16), (-(crc * bi + cic * br)).astype(bf16)], axis=0)
    bu = lax.dot_general(x_ref[...], bcat, NT, preferred_element_type=f32)
    for n in range(2 * NG):
        bu_ref[n] = bu[:, n * 128:(n + 1) * 128]

    post(3, r3)
    kt = jnp.concatenate(kts, axis=1)
    kmax = jnp.sqrt(jnp.max(jnp.sum(kt * kt, axis=0, keepdims=True), axis=1, keepdims=True))
    km16 = (kmax * (1.0 / 16.0)).astype(bf16).astype(f32)
    TT = jnp.concatenate([kt, jnp.broadcast_to(km16, (16, S)), jnp.zeros((96, S), f32)], axis=0).T
    k_ref[...] = pltpu.bitcast(TT.astype(bf16), u32)
    for ka_ref in ka_refs:
        ka_ref[T_KC] = jnp.broadcast_to(km16 * 16.0, (8, 128))
        ka_ref[T_ANC] = jnp.zeros((8, 128), f32)
    bu_ref[2 * NG, 0:8, :] = jnp.zeros((8, 128), f32)
    kv = TT[NC * CK:, :]
    kvb = [kv[b * 8:b * 8 + 8] for b in range(CK // 8)]
    for d in range(DH):
        for b in range(CK // 8):
            kbv = jnp.broadcast_to(kvb[b][:, d:d + 1], (8, 128))
            for ka_ref in ka_refs:
                ka_ref[T_KB + d * 16 + b] = kbv

    car_ref[...] = jnp.zeros(car_ref.shape, f32)
    ok_ref[...] = jnp.ones(ok_ref.shape, f32)
    for n in range(4):
        ka_refs[(NIT - 1) % 2][T_PVB + ((NIT - 1) // 2) * PPI + n] = jnp.zeros((8, 128), f32)
    pc_ref[...] = jnp.zeros(pc_ref.shape, u32)

    PER = S // TS

    def scan_block(ii, b, carry):
        gi = lax.shift_right_logical(ii, PER.bit_length() - 1)
        t0 = (ii & (PER - 1)) * TS

        def cst(n):
            return cst_ref[n * NG + gi]
        if b == 0:
            cr, ci, prev = car_ref[gi], car_ref[NG + gi], None
        else:
            cr, ci, prev = carry
        rs = pl.ds(pl.multiple_of(t0 + b * 8, 8), 8)
        tr, ti = _cmul(cst(0), cst(1), cr, ci)
        ur = bu_ref[gi, rs, :] + tr
        ui = bu_ref[NG + gi, rs, :] + ti
        for n, sh in enumerate((1, 2, 4)):
            tr, ti = _cmul(cst(2 + 2 * n), cst(3 + 2 * n), pltpu.roll(ur, sh, 0), pltpu.roll(ui, sh, 0))
            ur = ur + tr
            ui = ui + ti
        cr = jnp.broadcast_to(ur[7:8], (8, 128))
        ci = jnp.broadcast_to(ui[7:8], (8, 128))
        if b % 2 == 1:
            hs = pl.ds(pl.multiple_of(t0 + (b - 1) * 8, 16), 16)
            h_ref[gi, hs, :] = jnp.concatenate([prev[0], ur], axis=0).astype(bf16)
            h_ref[NG + gi, hs, :] = jnp.concatenate([prev[1], ui], axis=0).astype(bf16)
        if b == TS // 8 - 1:
            car_ref[gi] = cr
            car_ref[NG + gi] = ci
        return cr, ci, (ur, ui)

    def ld_k(c):
        return pltpu.bitcast(k_ref[c * CK // 2:(c + 1) * CK // 2, :], bf16)[:, :32]

    def ld_vt(c):
        return pltpu.bitcast(vt_ref[:, c * CK:(c + 1) * CK], bf16)

    def pv_ld(r, o):
        return ka_refs[r % 2][T_PVB + (r // 2) * PPI + o]

    def pv_st(r, o, z, v):
        ka_refs[r % 2][z + (T_PVB + (r // 2) * PPI + o)] = v

    def finish(h, j, r, acc, l):
        lv = jnp.concatenate([pv_ld(r, n) for n in range(4)], axis=1)
        lsum = jnp.sum(l + lv, axis=0, keepdims=True)
        okv = jnp.where((lsum > L_LO) & (lsum < L_HI), 1.0, 0.0)
        for n in range(4):
            ok_ref[n] = jnp.minimum(ok_ref[n], okv[:, n * 128:(n + 1) * 128])
        ot_ref[pl.ds(pl.multiple_of(h * 16, 16), 16), j * BQ:(j + 1) * BQ] = (
            acc * ((1.0 / lsum) * (1.0 / V_UP))).astype(bf16)

    def pc_slice(n):
        return slice(n * CK // 2, (n + 1) * CK // 2)

    def pvv(r):
        pb = jnp.concatenate([
            jnp.concatenate([pltpu.bitcast(lax.bitcast_convert_type(pv_ld(r, 4 + rb * 4 + qt), u32), bf16)
                             for qt in range(4)], axis=1) for rb in range(8)], axis=0)
        return jnp.dot(ld_vt(NC), pb, preferred_element_type=f32)

    def piece(h, j, r, u, z):
        kp, qt = u // 4, u % 4
        kbs = (2 * kp, 2 * kp + 1)
        ka_ref = ka_refs[r % 2]
        cs = slice(j * BQ + qt * 128, j * BQ + (qt + 1) * 128)
        m0 = ka_ref[T_KC] * qf_ref[h, 16:24, cs]
        accs = [m0, m0]
        for d in range(DH):
            if d % 8 == 0:
                q8 = qf_ref[h, d:d + 8, cs]
            qrow = jnp.broadcast_to(q8[d % 8:d % 8 + 1], (8, 128))
            for n, kb in enumerate(kbs):
                accs[n] = accs[n] + ka_ref[T_KB + d * 16 + kb] * qrow
        ps = [jnp.exp2(a) for a in accs]
        ls = ps[0] + ps[1]
        if kp > 0:
            ls = ls + pv_ld(r, qt)
        pv_st(r, qt, z, ls)
        pk = pltpu.bitcast(jnp.concatenate(ps, axis=0).astype(bf16), u32)
        pv_st(r, 4 + kp * 4 + qt, z, lax.bitcast_convert_type(pk, f32))

    NB = NIT * NC
    events = {}
    for n in range(FREE, NIT * NP):
        g, rb = _slot_of((n - FREE) * PSP)
        events.setdefault(g, []).append((rb, 0, n))
    for n in range(TS // 8):
        g, rb = _slot_of(SOFF + n * SSP)
        events.setdefault(g, []).append((rb, 1, n))

    def attn_body(ii, carry):
        acc, l = carry
        z = lax.shift_right_logical(ii, 16)
        qts = {}

        def getq(r):
            if r not in qts:
                h = ii * HPI + r // NQ
                j = r % NQ
                qts[r] = qa_ref[pl.ds(pl.multiple_of(h * 32, 32), 32), j * BQ:(j + 1) * BQ]
            return qts[r]
        pend = {}
        lnext = None
        scar = None
        for n in range(FREE):
            piece(ii * HPI, 0, 0, n, z)
        for g in range(NB):
            r, c = g // NC, g % NC
            s = jnp.dot(ld_k(c), getq(r), preferred_element_type=f32)
            if g >= NB - LAG:
                p = jnp.exp2(s)
                ls = jnp.sum(p.reshape(CK // 8, 8, BQ), axis=0)
                lnext = ls if lnext is None else lnext + ls
                pc_ref[pc_slice(g - (NB - LAG)), :] = pltpu.bitcast(p.astype(bf16), u32)
            else:
                pend[g] = s
            gp = g - LAG
            rp, cpos = gp // NC, gp % NC
            if gp < 0:
                pb = pltpu.bitcast(pc_ref[pc_slice(gp + LAG), :], bf16)
            else:
                p = jnp.exp2(pend.pop(gp))
                ls = jnp.sum(p.reshape(CK // 8, 8, BQ), axis=0)
                l = ls if l is None else l + ls
                pb = p.astype(bf16)
            o = jnp.dot(ld_vt(cpos), pb, preferred_element_type=f32)
            acc = o if acc is None else acc + o
            if cpos == NC - 1:
                if rp >= 0:
                    acc = acc + pvv(rp)
                finish(jnp.maximum(ii * HPI + rp // NQ, 0), rp % NQ, rp % NIT, acc, l)
                l = acc = None
            for rb, kind, n in sorted(events.get(g, [])):
                anc = s[rb * 8:(rb + 1) * 8, 0:128]
                if kind == 0:
                    rr = n // NP
                    ka_refs[rr % 2][z + T_ANC] = anc
                    piece(ii * HPI + rr // NQ, rr % NQ, rr, n % NP, z)
                else:
                    bu_ref[2 * NG, 0:8, :] = anc
                    scar = scan_block(ii, n, scar)
        acc = acc + pvv(NIT - 1)
        return acc, l + lnext

    acc, l = lax.fori_loop(0, NLOOP, attn_body, (jnp.zeros((16, BQ), f32), jnp.ones((8, BQ), f32)))
    for n in range(LAG):
        acc = acc + jnp.dot(ld_vt(NC - LAG + n), pltpu.bitcast(pc_ref[pc_slice(n), :], bf16),
                            preferred_element_type=f32)
    finish(H - 1, NQ - 1, NIT - 1, acc, l)

    @pl.when(jnp.min(ok_ref[...]) < 0.5)
    def _fallback():
        FK = 256

        def fb(i, c):
            h = lax.shift_right_logical(i, 4)
            cs = pl.ds(pl.multiple_of((i & 15) * 128, 128), 128)
            qt = qa_ref[pl.ds(pl.multiple_of(h * 32, 32), 16), cs]

            def scores(kc):
                ks = pl.ds(pl.multiple_of(kc * (FK // 2), FK // 2), FK // 2)
                kf = pltpu.bitcast(k_ref[ks, :], bf16)[:, :16]
                return jnp.dot(kf, qt, preferred_element_type=f32)

            def pass1(kc, m):
                return jnp.maximum(m, jnp.max(scores(kc), axis=0, keepdims=True))
            m = lax.fori_loop(0, S // FK, pass1, jnp.full((1, 128), -jnp.inf, f32))

            def pass2(kc, carry):
                ls, o = carry
                p = jnp.exp2(scores(kc) - m)
                vs = pltpu.bitcast(vt_ref[:, pl.ds(pl.multiple_of(kc * FK, FK), FK)], bf16)
                return (ls + jnp.sum(p, axis=0, keepdims=True),
                        o + jnp.dot(vs, p.astype(bf16), preferred_element_type=f32))
            ls, o = lax.fori_loop(0, S // FK, pass2, (jnp.zeros((1, 128), f32), jnp.zeros((16, 128), f32)))
            ot_ref[pl.ds(pl.multiple_of(h * 16, 16), 16), cs] = (o * ((1.0 / ls) * (1.0 / V_UP))).astype(bf16)
            return c
        lax.fori_loop(0, H * (S // 128), fb, 0)

    wait(c_cps)
    ccat = jnp.concatenate([cre_ref[...], cim_ref[...]], axis=1)
    wo = wo_ref[...]
    dskip = dskip_ref[...].reshape(1, D).astype(f32)
    gate = gate_ref[...].reshape(1, D).astype(f32)
    r0 = 0
    for RF in FCH:
        rs = slice(r0, r0 + RF)
        hc = jnp.concatenate([h_ref[n, rs, :] for n in range(2 * NG)], axis=1)
        yb = lax.dot_general(hc, ccat, NT, preferred_element_type=f32)
        ya = lax.dot_general(ot_ref[:, rs], wo, TN, preferred_element_type=f32)
        xf = x_ref[rs, :].astype(f32)
        g = jax.nn.sigmoid(jnp.sum(xf * gate, axis=1, keepdims=True))
        yb = yb + xf * dskip
        o_ref[rs, :] = g * ya + (1.0 - g) * yb
        pltpu.make_async_copy(o_ref.at[pl.ds(r0, RF)], o_hbm.at[pl.ds(r0, RF)], osem.at[0]).start()
        r0 += RF
    pltpu.make_async_copy(o_ref, o_hbm, osem.at[0]).wait()


@jax.jit
def pallas_gated_mix__grouped_kv_mqa__ssm_conv_s5__prompt_kernel(
    A_x, A_wq, A_wk, A_wv, A_wo, B_x, B_Lambda_re, B_Lambda_im, B_B_re, B_B_im, B_C_re, B_C_im,
    B_log_dt, B_Dskip, gate_w,
):
    del B_x
    vm = pltpu.VMEM
    out = pl.pallas_call(
        _kernel,
        out_shape=jax.ShapeDtypeStruct((S, D), f32),
        in_specs=[pl.BlockSpec(memory_space=pl.ANY)] * 14,
        out_specs=pl.BlockSpec(memory_space=pl.ANY),
        scratch_shapes=[
            vm((S, D), bf16), vm((D, D), bf16), vm((DH, D), bf16), vm((DH, D), bf16), vm((D, D), bf16),
            vm((P,), bf16), vm((P,), bf16), vm((P, D), bf16), vm((P, D), bf16), vm((D, P), bf16), vm((D, P), bf16),
            vm((P,), bf16), vm((D,), bf16), vm((D,), bf16), vm((S, D), f32),
            vm((H * 32, S), bf16),
            vm((H, 24, S), f32),
            vm((S // 2, 128), u32),
            vm((8, S), u32),
            vm((2 * NG + 1, S, 128), f32),
            vm((2 * NG, S, 128), bf16),
            vm((D, S), bf16),
            vm((8 * NG, 8, 128), f32),
            [vm((T_END, 8, 128), f32)] * 2,
            vm((2 * NG, 8, 128), f32),
            vm((4, 8, 128), f32),
            vm((LAG * CK // 2, BQ), u32),
            pltpu.SemaphoreType.DMA((17,)), pltpu.SemaphoreType.DMA((1,)),
        ],
        compiler_params=pltpu.CompilerParams(vmem_limit_bytes=100 * 2 ** 20),
        name="gmix",
    )(A_x.reshape(S, D), A_wq, A_wk.T, A_wv.T, A_wo, B_Lambda_re, B_Lambda_im, B_B_re, B_B_im,
      B_C_re, B_C_im, B_log_dt, B_Dskip, gate_w)
    return out.reshape(1, S, D)
```

```python
import jax
import jax.numpy as jnp
from jax import lax
import jax.experimental.pallas as pl
import jax.experimental.pallas.tpu as pltpu

S = 2048
D = 512
H = 32
DH = 16
P = 512
BQ = 512
CK = 128
HPI = 2
LAG = 2
XB = 512
FCH = (128,) + (256,) * 7 + (64, 64)

LOG2E = 1.4426950408889634
QSCALE = (DH ** -0.5) * LOG2E
L_LO = 2.0 ** -64
L_HI = 2.0 ** 12
V_UP = 2.0 ** 40

bf16 = jnp.bfloat16
f32 = jnp.float32
u32 = jnp.uint32

NT = (((1,), (1,)), ((), ()))
TN = (((0,), (0,)), ((), ()))

NQ = S // BQ
NCA = S // CK
NC = NCA - 1
NIT = NQ * HPI
NLOOP = H // HPI
NG = P // 128
TS = S * NG // NLOOP
NP = 32

T_KC = 0
T_ANC = 1
T_KB = 2
T_PVB = T_KB + 256
PPI = 36
T_END = T_PVB + (NIT // 2) * PPI

CHT = 136
PSP = NIT * NC * CHT / (NP * NIT)
FREE = 2
SSP = NIT * NC * CHT / (TS // 8)
SOFF = 112


def _cmul(ar, ai, br, bi):
    return ar * br - ai * bi, ar * bi + ai * br


def _slot_of(t):
    g = int(t // CHT)
    return g, min(int((t - g * CHT) // 8), 15)


def _kernel(x_hbm, wq_hbm, wkT_hbm, wvT_hbm, wo_hbm, lre_hbm, lim_hbm, bre_hbm, bim_hbm,
            cre_hbm, cim_hbm, ldt_hbm, dskip_hbm, gate_hbm, o_hbm,
            x_ref, wq_ref, wkT_ref, wvT_ref, wo_ref, lre_ref, lim_ref, bre_ref, bim_ref,
            cre_ref, cim_ref, ldt_ref, dskip_ref, gate_ref, o_ref,
            qa_ref, k_ref, vt_ref, bu_ref, h_ref, ot_ref, cst_ref, ka_refs, car_ref, ok_ref, pc_ref,
            isem, osem):
    def cp(src, dst, n):
        return pltpu.make_async_copy(src, dst, isem.at[n])
    x_cps = [cp(x_hbm.at[pl.ds(j * XB, XB)], x_ref.at[pl.ds(j * XB, XB)], j) for j in range(S // XB)]
    wq_cp = cp(wq_hbm, wq_ref, 4)
    small = [cp(wkT_hbm, wkT_ref, 5), cp(wvT_hbm, wvT_ref, 6),
             cp(lre_hbm, lre_ref, 8), cp(lim_hbm, lim_ref, 9), cp(ldt_hbm, ldt_ref, 10)]
    b_cps = [cp(bre_hbm, bre_ref, 12), cp(bim_hbm, bim_ref, 13)]
    c_cps = [cp(cre_hbm, cre_ref, 14), cp(cim_hbm, cim_ref, 15), cp(wo_hbm, wo_ref, 16),
             cp(dskip_hbm, dskip_ref, 11), cp(gate_hbm, gate_ref, 7)]

    def start(cs):
        for c in cs:
            c.start()

    def wait(cs):
        for c in cs:
            c.wait()

    start(small + [wq_cp] + x_cps + b_cps)
    wait(small + [wq_cp])

    wT = jnp.concatenate([wkT_ref[...], wvT_ref[...], wq_ref[...].T], axis=0)
    kts = []

    def proj(j):
        return lax.dot_general(wT, x_ref[j * XB:(j + 1) * XB, :], NT, preferred_element_type=f32)

    def post(j, r):
        cs = slice(j * XB, (j + 1) * XB)
        qs = r[2 * DH:] * QSCALE
        for h in range(H):
            qf = qs[h * DH:(h + 1) * DH]
            n2 = jnp.sum(qf * qf, axis=0, keepdims=True)
            nn = n2 * lax.rsqrt(n2 + 1e-30) * (-1.0 - 2.0 ** -7)
            qh = qf.astype(bf16)
            nh = jnp.broadcast_to(nn, (16, XB)).astype(bf16)
            qa_ref[h * 32:h * 32 + 16, cs] = qh
            qa_ref[h * 32 + 16:h * 32 + 32, cs] = nh
        kts.append(r[:DH].astype(bf16).astype(f32))
        vt_ref[:, cs] = pltpu.bitcast((r[DH:2 * DH] * V_UP).astype(bf16), u32)

    def ssm_consts():
        lre = lre_ref[...].reshape(1, P).astype(f32)
        lim = lim_ref[...].reshape(1, P).astype(f32)
        dt = jnp.exp(ldt_ref[...].reshape(1, P).astype(f32)).astype(bf16).astype(f32)
        row = lax.broadcasted_iota(jnp.int32, (8, P), 0)
        kk = jnp.where(row == 0, 1, jnp.where(row == 1, 2, 4)).astype(f32)
        mag = jnp.exp(kk * (dt * lre))
        ang = kk * (dt * lim)
        pwr = mag * jnp.cos(ang)
        pwi = mag * jnp.sin(ang)
        l1r, l1i = pwr[0:1], pwi[0:1]
        den = 2.0 / (lre * lre + lim * lim)
        nr = l1r - 1.0
        cfr = (nr * lre + l1i * lim) * den
        cfi = (l1i * lre - nr * lim) * den
        consts = [
            jnp.where(row == 0, jnp.broadcast_to(l1r, (8, P)), 0.0),
            jnp.where(row == 0, jnp.broadcast_to(-l1i, (8, P)), 0.0),
        ]
        for sh, src in ((1, 0), (2, 1), (4, 2)):
            consts.append(jnp.where(row >= sh, jnp.broadcast_to(pwr[src:src + 1], (8, P)), 0.0))
            consts.append(jnp.where(row >= sh, jnp.broadcast_to(-pwi[src:src + 1], (8, P)), 0.0))
        for n, cv in enumerate(consts):
            for gi in range(NG):
                cst_ref[n * NG + gi] = cv[:, gi * 128:(gi + 1) * 128]
        cfT = jnp.concatenate([jnp.broadcast_to(cfr, (64, P)), jnp.broadcast_to(cfi, (64, P))], axis=0).T
        return cfT[:, 0:1], cfT[:, 64:65]

    crc, cic = ssm_consts()
    wait(x_cps[:1])
    post(0, proj(0))
    wait(x_cps[1:3])
    post(1, proj(1))
    post(2, proj(2))
    wait(x_cps[3:] + b_cps)
    start(c_cps)
    r3 = proj(3)

    br = bre_ref[...].astype(f32)
    bi = bim_ref[...].astype(f32)
    bcat = jnp.concatenate([(crc * br - cic * bi).astype(bf16), (-(crc * bi + cic * br)).astype(bf16)], axis=0)
    bu = lax.dot_general(x_ref[...], bcat, NT, preferred_element_type=f32)
    for n in range(2 * NG):
        bu_ref[n] = bu[:, n * 128:(n + 1) * 128]

    post(3, r3)
    kt = jnp.concatenate(kts, axis=1)
    kmax = jnp.sqrt(jnp.max(jnp.sum(kt * kt, axis=0, keepdims=True), axis=1, keepdims=True))
    km16 = (kmax * (1.0 / 16.0)).astype(bf16).astype(f32)
    TT = jnp.concatenate([kt, jnp.broadcast_to(km16, (16, S)), jnp.zeros((96, S), f32)], axis=0).T
    k_ref[...] = pltpu.bitcast(TT.astype(bf16), u32)
    for ka_ref in ka_refs:
        ka_ref[T_KC] = jnp.broadcast_to(km16 * 16.0, (8, 128))
        ka_ref[T_ANC] = jnp.zeros((8, 128), f32)
    bu_ref[2 * NG, 0:8, :] = jnp.zeros((8, 128), f32)
    kv = TT[NC * CK:, :]
    kvb = [kv[b * 8:b * 8 + 8] for b in range(CK // 8)]
    for d in range(DH):
        for b in range(CK // 8):
            kbv = jnp.broadcast_to(kvb[b][:, d:d + 1], (8, 128))
            for ka_ref in ka_refs:
                ka_ref[T_KB + d * 16 + b] = kbv

    car_ref[...] = jnp.zeros(car_ref.shape, f32)
    ok_ref[...] = jnp.ones(ok_ref.shape, f32)
    for n in range(4):
        ka_refs[(NIT - 1) % 2][T_PVB + ((NIT - 1) // 2) * PPI + n] = jnp.zeros((8, 128), f32)
    pc_ref[...] = jnp.zeros(pc_ref.shape, u32)

    PER = S // TS

    def scan_block(ii, b, carry):
        gi = lax.shift_right_logical(ii, PER.bit_length() - 1)
        t0 = (ii & (PER - 1)) * TS

        def cst(n):
            return cst_ref[n * NG + gi]
        if b == 0:
            cr, ci, prev = car_ref[gi], car_ref[NG + gi], None
        else:
            cr, ci, prev = carry
        rs = pl.ds(pl.multiple_of(t0 + b * 8, 8), 8)
        tr, ti = _cmul(cst(0), cst(1), cr, ci)
        ur = bu_ref[gi, rs, :] + tr
        ui = bu_ref[NG + gi, rs, :] + ti
        for n, sh in enumerate((1, 2, 4)):
            tr, ti = _cmul(cst(2 + 2 * n), cst(3 + 2 * n), pltpu.roll(ur, sh, 0), pltpu.roll(ui, sh, 0))
            ur = ur + tr
            ui = ui + ti
        cr = jnp.broadcast_to(ur[7:8], (8, 128))
        ci = jnp.broadcast_to(ui[7:8], (8, 128))
        if b % 2 == 1:
            hs = pl.ds(pl.multiple_of(t0 + (b - 1) * 8, 16), 16)
            h_ref[gi, hs, :] = jnp.concatenate([prev[0], ur], axis=0).astype(bf16)
            h_ref[NG + gi, hs, :] = jnp.concatenate([prev[1], ui], axis=0).astype(bf16)
        if b == TS // 8 - 1:
            car_ref[gi] = cr
            car_ref[NG + gi] = ci
        return cr, ci, (ur, ui)

    def ld_k(c):
        return pltpu.bitcast(k_ref[c * CK // 2:(c + 1) * CK // 2, :], bf16)[:, :32]

    def ld_vt(c):
        return pltpu.bitcast(vt_ref[:, c * CK:(c + 1) * CK], bf16)

    def pv_ld(r, o):
        return ka_refs[r % 2][T_PVB + (r // 2) * PPI + o]

    def pv_st(r, o, z, v):
        ka_refs[r % 2][z + (T_PVB + (r // 2) * PPI + o)] = v

    def finish(h, j, r, acc, l):
        lv = jnp.concatenate([pv_ld(r, n) for n in range(4)], axis=1)
        lsum = jnp.sum(l + lv, axis=0, keepdims=True)
        okv = jnp.where((lsum > L_LO) & (lsum < L_HI), 1.0, 0.0)
        for n in range(4):
            ok_ref[n] = jnp.minimum(ok_ref[n], okv[:, n * 128:(n + 1) * 128])
        ot_ref[pl.ds(pl.multiple_of(h * 16, 16), 16), j * BQ:(j + 1) * BQ] = (
            acc * ((1.0 / lsum) * (1.0 / V_UP))).astype(bf16)

    def pc_slice(n):
        return slice(n * CK // 2, (n + 1) * CK // 2)

    def pvv(r):
        pb = jnp.concatenate([
            jnp.concatenate([pltpu.bitcast(lax.bitcast_convert_type(pv_ld(r, 4 + rb * 4 + qt), u32), bf16)
                             for qt in range(4)], axis=1) for rb in range(8)], axis=0)
        return jnp.dot(ld_vt(NC), pb, preferred_element_type=f32)

    def piece(qv, r, u, z):
        kp, qt = u // 4, u % 4
        kbs = (2 * kp, 2 * kp + 1)
        ka_ref = ka_refs[r % 2]
        qf = qv[:, qt * 128:(qt + 1) * 128].astype(f32)
        m0 = ka_ref[T_KC] * qf[16:24]
        accs = [m0, m0]
        for d in range(DH):
            qrow = jnp.broadcast_to(qf[d:d + 1], (8, 128))
            for n, kb in enumerate(kbs):
                accs[n] = accs[n] + ka_ref[T_KB + d * 16 + kb] * qrow
        ps = [jnp.exp2(a) for a in accs]
        ls = ps[0] + ps[1]
        if kp > 0:
            ls = ls + pv_ld(r, qt)
        pv_st(r, qt, z, ls)
        pk = pltpu.bitcast(jnp.concatenate(ps, axis=0).astype(bf16), u32)
        pv_st(r, 4 + kp * 4 + qt, z, lax.bitcast_convert_type(pk, f32))

    NB = NIT * NC
    events = {}
    for n in range(FREE, NIT * NP):
        g, rb = _slot_of((n - FREE) * PSP)
        events.setdefault(g, []).append((rb, 0, n))
    for n in range(TS // 8):
        g, rb = _slot_of(SOFF + n * SSP)
        events.setdefault(g, []).append((rb, 1, n))

    def attn_body(ii, carry):
        acc, l = carry
        z = lax.shift_right_logical(ii, 16)
        qts = {}

        def getq(r):
            if r not in qts:
                h = ii * HPI + r // NQ
                j = r % NQ
                qts[r] = qa_ref[pl.ds(pl.multiple_of(h * 32, 32), 32), j * BQ:(j + 1) * BQ]
            return qts[r]
        pend = {}
        lnext = None
        scar = None
        for n in range(FREE):
            piece(getq(0), 0, n, z)
        for g in range(NB):
            r, c = g // NC, g % NC
            s = jnp.dot(ld_k(c), getq(r), preferred_element_type=f32)
            if g >= NB - LAG:
                p = jnp.exp2(s)
                ls = jnp.sum(p.reshape(CK // 8, 8, BQ), axis=0)
                lnext = ls if lnext is None else lnext + ls
                pc_ref[pc_slice(g - (NB - LAG)), :] = pltpu.bitcast(p.astype(bf16), u32)
            else:
                pend[g] = s
            gp = g - LAG
            rp, cpos = gp // NC, gp % NC
            if gp < 0:
                pb = pltpu.bitcast(pc_ref[pc_slice(gp + LAG), :], bf16)
            else:
                p = jnp.exp2(pend.pop(gp))
                ls = jnp.sum(p.reshape(CK // 8, 8, BQ), axis=0)
                l = ls if l is None else l + ls
                pb = p.astype(bf16)
            o = jnp.dot(ld_vt(cpos), pb, preferred_element_type=f32)
            acc = o if acc is None else acc + o
            if cpos == NC - 1:
                if rp >= 0:
                    acc = acc + pvv(rp)
                finish(jnp.maximum(ii * HPI + rp // NQ, 0), rp % NQ, rp % NIT, acc, l)
                l = acc = None
            for rb, kind, n in sorted(events.get(g, [])):
                anc = s[rb * 8:(rb + 1) * 8, 0:128]
                if kind == 0:
                    rr = n // NP
                    ka_refs[rr % 2][z + T_ANC] = anc
                    piece(getq(rr), rr, n % NP, z)
                else:
                    bu_ref[2 * NG, 0:8, :] = anc
                    scar = scan_block(ii, n, scar)
        acc = acc + pvv(NIT - 1)
        return acc, l + lnext

    acc, l = lax.fori_loop(0, NLOOP, attn_body, (jnp.zeros((16, BQ), f32), jnp.ones((8, BQ), f32)))
    for n in range(LAG):
        acc = acc + jnp.dot(ld_vt(NC - LAG + n), pltpu.bitcast(pc_ref[pc_slice(n), :], bf16),
                            preferred_element_type=f32)
    finish(H - 1, NQ - 1, NIT - 1, acc, l)

    @pl.when(jnp.min(ok_ref[...]) < 0.5)
    def _fallback():
        FK = 256

        def fb(i, c):
            h = lax.shift_right_logical(i, 4)
            cs = pl.ds(pl.multiple_of((i & 15) * 128, 128), 128)
            qt = qa_ref[pl.ds(pl.multiple_of(h * 32, 32), 16), cs]

            def scores(kc):
                ks = pl.ds(pl.multiple_of(kc * (FK // 2), FK // 2), FK // 2)
                kf = pltpu.bitcast(k_ref[ks, :], bf16)[:, :16]
                return jnp.dot(kf, qt, preferred_element_type=f32)

            def pass1(kc, m):
                return jnp.maximum(m, jnp.max(scores(kc), axis=0, keepdims=True))
            m = lax.fori_loop(0, S // FK, pass1, jnp.full((1, 128), -jnp.inf, f32))

            def pass2(kc, carry):
                ls, o = carry
                p = jnp.exp2(scores(kc) - m)
                vs = pltpu.bitcast(vt_ref[:, pl.ds(pl.multiple_of(kc * FK, FK), FK)], bf16)
                return (ls + jnp.sum(p, axis=0, keepdims=True),
                        o + jnp.dot(vs, p.astype(bf16), preferred_element_type=f32))
            ls, o = lax.fori_loop(0, S // FK, pass2, (jnp.zeros((1, 128), f32), jnp.zeros((16, 128), f32)))
            ot_ref[pl.ds(pl.multiple_of(h * 16, 16), 16), cs] = (o * ((1.0 / ls) * (1.0 / V_UP))).astype(bf16)
            return c
        lax.fori_loop(0, H * (S // 128), fb, 0)

    wait(c_cps)
    ccat = jnp.concatenate([cre_ref[...], cim_ref[...]], axis=1)
    wo = wo_ref[...]
    dskip = dskip_ref[...].reshape(1, D).astype(f32)
    gate = gate_ref[...].reshape(1, D).astype(f32)
    r0 = 0
    for RF in FCH:
        rs = slice(r0, r0 + RF)
        hc = jnp.concatenate([h_ref[n, rs, :] for n in range(2 * NG)], axis=1)
        yb = lax.dot_general(hc, ccat, NT, preferred_element_type=f32)
        ya = lax.dot_general(ot_ref[:, rs], wo, TN, preferred_element_type=f32)
        xf = x_ref[rs, :].astype(f32)
        g = jax.nn.sigmoid(jnp.sum(xf * gate, axis=1, keepdims=True))
        yb = yb + xf * dskip
        o_ref[rs, :] = g * ya + (1.0 - g) * yb
        pltpu.make_async_copy(o_ref.at[pl.ds(r0, RF)], o_hbm.at[pl.ds(r0, RF)], osem.at[0]).start()
        r0 += RF
    pltpu.make_async_copy(o_ref, o_hbm, osem.at[0]).wait()


@jax.jit
def pallas_gated_mix__grouped_kv_mqa__ssm_conv_s5__prompt_kernel(
    A_x, A_wq, A_wk, A_wv, A_wo, B_x, B_Lambda_re, B_Lambda_im, B_B_re, B_B_im, B_C_re, B_C_im,
    B_log_dt, B_Dskip, gate_w,
):
    del B_x
    vm = pltpu.VMEM
    out = pl.pallas_call(
        _kernel,
        out_shape=jax.ShapeDtypeStruct((S, D), f32),
        in_specs=[pl.BlockSpec(memory_space=pl.ANY)] * 14,
        out_specs=pl.BlockSpec(memory_space=pl.ANY),
        scratch_shapes=[
            vm((S, D), bf16), vm((D, D), bf16), vm((DH, D), bf16), vm((DH, D), bf16), vm((D, D), bf16),
            vm((P,), bf16), vm((P,), bf16), vm((P, D), bf16), vm((P, D), bf16), vm((D, P), bf16), vm((D, P), bf16),
            vm((P,), bf16), vm((D,), bf16), vm((D,), bf16), vm((S, D), f32),
            vm((H * 32, S), bf16),
            vm((S // 2, 128), u32),
            vm((8, S), u32),
            vm((2 * NG + 1, S, 128), f32),
            vm((2 * NG, S, 128), bf16),
            vm((D, S), bf16),
            vm((8 * NG, 8, 128), f32),
            [vm((T_END, 8, 128), f32)] * 2,
            vm((2 * NG, 8, 128), f32),
            vm((4, 8, 128), f32),
            vm((LAG * CK // 2, BQ), u32),
            pltpu.SemaphoreType.DMA((17,)), pltpu.SemaphoreType.DMA((1,)),
        ],
        compiler_params=pltpu.CompilerParams(vmem_limit_bytes=100 * 2 ** 20),
        name="gmix",
    )(A_x.reshape(S, D), A_wq, A_wk.T, A_wv.T, A_wo, B_Lambda_re, B_Lambda_im, B_B_re, B_B_im,
      B_C_re, B_C_im, B_log_dt, B_Dskip, gate_w)
    return out.reshape(1, S, D)
```
